```python
import jax
import jax.numpy as jnp

def _softmax(x, axis=-1):
    return jax.nn.softmax(x, axis=axis)

def _gelu(x):
    return jax.nn.gelu(x, approximate=True)

def _silu(x):
    return jax.nn.silu(x)

def _sigmoid(x):
    return jax.nn.sigmoid(x)

def _layernorm(x, axis=-1, eps=1e-05):
    m = jnp.mean(x, axis=axis, keepdims=True)
    v = jnp.var(x, axis=axis, keepdims=True)
    return (x - m) / jnp.sqrt(v + eps)

def _scatter_add(tgt, idx, src, axis=0):
    return tgt.at[idx].add(src)

def _segment_sum(src, seg, n):
    return jax.ops.segment_sum(src, seg, n)

class _Rng:

    def __init__(self, key):
        self._k = key

    def _next(self):
        self._k, sub = jax.random.split(self._k)
        return sub

    def normal(self, shape):
        return jax.random.normal(self._next(), shape, dtype=jnp.bfloat16)

    def randint(self, lo, hi, shape):
        return jax.random.randint(self._next(), shape, lo, hi, dtype=jnp.int32)

    def uniform(self, shape, lo=0.0, hi=1.0):
        return jax.random.uniform(self._next(), shape, jnp.bfloat16, lo, hi)

    def permutation(self, n):
        return jax.random.permutation(self._next(), n)
kernel_name = 'adaLN_cond__gqa_block_cached__moe_arch_mod__decode'

def setup_inputs():
    _rng = _Rng(jax.random.key(int.from_bytes(__import__("os").urandom(4), "little")))
    _w = lambda a: (lambda t: t.astype(jnp.bfloat16) if jnp.issubdtype(t.dtype, jnp.floating) else t)(jnp.asarray(a))

    def _A_setup():
        B, Sq, D = (4, 1, 512)
        Hq, Hkv, Sk, Dh = (32, 32, 8192, 128)
        assert Hq % Hkv == 0, (Hq, Hkv)
        return {'x': _w((lambda *s: _rng.normal(s) * 0.05)(B, Sq, D)), 'k_cache': _w((lambda *s: _rng.normal(s) * 0.05)(B, Hkv, Sk, Dh)), 'v_cache': _w((lambda *s: _rng.normal(s) * 0.05)(B, Hkv, Sk, Dh)), 'wq': _w((lambda *s: _rng.normal(s) * 0.05)(D, Hq * Dh) * D ** (-0.5)), 'wo': _w((lambda *s: _rng.normal(s) * 0.05)(Hq * Dh, D) * (Hq * Dh) ** (-0.5))}
    _A_in = _A_setup()

    def _B_setup():
        B, S, D, F, C = (4, 1, 512, 1376, 1)
        return {'x': _w((lambda *s: _rng.normal(s) * 0.05)(B, S, D)), 'w_r': _w((lambda *s: _rng.normal(s) * 0.05)(D)), 'w_gate': _w((lambda *s: _rng.normal(s) * 0.05)(D, F)), 'w_up': _w((lambda *s: _rng.normal(s) * 0.05)(D, F)), 'w_down': _w((lambda *s: _rng.normal(s) * 0.05)(F, D))}
    _B_in = _B_setup()
    return {'A_x': _A_in['x'], 'A_k_cache': _A_in['k_cache'], 'A_v_cache': _A_in['v_cache'], 'A_wq': _A_in['wq'], 'A_wo': _A_in['wo'], 'B_x': _B_in['x'], 'B_w_r': _B_in['w_r'], 'B_w_gate': _B_in['w_gate'], 'B_w_up': _B_in['w_up'], 'B_w_down': _B_in['w_down'], 'c': _w((lambda *s: _rng.normal(s) * 0.05)(4, 512)), 'w_mod': _w((lambda *s: _rng.normal(s) * 0.05)(512, 6 * 512) * 512 ** (-0.5))}

def reference(A_x, A_k_cache, A_v_cache, A_wq, A_wo, B_x, B_w_r, B_w_gate, B_w_up, B_w_down, c, w_mod):

    def _A_ref(x, k_cache, v_cache, wq, wo):
        B, Sq, D = x.shape
        Hq, Dh = (32, 128)
        Hkv = k_cache.shape[1]
        rep = Hq // Hkv
        q = (lambda x, *d: x.transpose(*d))((x @ wq).reshape(B, Sq, Hq, Dh), 0, 2, 1, 3)
        k = jnp.repeat(k_cache, rep, axis=1)
        v = jnp.repeat(v_cache, rep, axis=1)
        scores = jnp.einsum('bhqd,bhkd->bhqk', q, k) * Dh ** (-0.5)
        p = _softmax(scores, axis=-1)
        o = jnp.einsum('bhqk,bhkd->bhqd', p, v)
        return (lambda x, *d: x.transpose(*d))(o, 0, 2, 1, 3).reshape(B, Sq, Hq * Dh) @ wo

    def _B_ref(x, w_r, w_gate, w_up, w_down):
        B, S, D = x.shape
        C = 1
        r = x @ w_r
        idx = jnp.argsort(-r, axis=-1)[:, :C]
        idx_e = jnp.repeat(idx.reshape(B, C, 1), D, axis=2)
        x_sel = jnp.take_along_axis(x, idx_e, axis=1)
        g = _silu(x_sel @ w_gate)
        u = x_sel @ w_up
        y = g * u @ w_down
        r_sel = _sigmoid(jnp.take_along_axis(r, idx, axis=1))
        y = y * r_sel.reshape(B, C, 1)
        b_off = (jnp.arange(B) * S).reshape(B, 1)
        flat_idx = (idx + b_off).reshape(B * C)
        zero = (x * 0.0).reshape(B * S, D)
        upd = _scatter_add(zero, flat_idx, y.reshape(B * C, D), axis=0)
        return x + upd.reshape(B, S, D)
    x = A_x
    mod = (_silu(c) @ w_mod).reshape(c.shape[0], 6, 1, -1)
    sa, ca, ga, sb, cb, gb = (mod[:, 0].copy(), mod[:, 1].copy(), mod[:, 2].copy(), mod[:, 3].copy(), mod[:, 4].copy(), mod[:, 5].copy())
    h = _layernorm(x, axis=-1) * (1 + ca) + sa
    x = x + ga * _A_ref(h, A_k_cache, A_v_cache, A_wq, A_wo)
    h = _layernorm(x, axis=-1) * (1 + cb) + sb
    x = x + gb * _B_ref(h, B_w_r, B_w_gate, B_w_up, B_w_down)
    return x
```

```python
import functools

import jax
import jax.numpy as jnp
import jax.experimental.pallas as pl
import jax.experimental.pallas.tpu as pltpu

B, D, HQ, SK, DH, FF = 4, 512, 32, 8192, 128, 1376
NSTEP = B * HQ
EPS = 1e-5


def _layernorm(x):
    m = jnp.mean(x, axis=-1, keepdims=True)
    d = x - m
    v = jnp.mean(d * d, axis=-1, keepdims=True)
    return d * jax.lax.rsqrt(v + EPS)


def _silu(x):
    return x * jax.nn.sigmoid(x)


def _dot(a, b):
    return jnp.dot(a, b, preferred_element_type=jnp.float32)


def _dot_nt(a, b):
    return jax.lax.dot_general(a, b, (((1,), (1,)), ((), ())), preferred_element_type=jnp.float32)


def _kernel(x_hbm, k_hbm, v_hbm, wq_hbm, wo_hbm, wr_hbm, wg_hbm, wu_hbm, wd_hbm, c_hbm, wm_hbm,
            out_ref,
            kbuf, vbuf, x_s, c_s, wr_s, wq_s, wo_s, wg_s, wu_s, wd_s, wm_s,
            q_s, mod_s, ksem, vsem, wsem, *, dist, rows, npiece, nodma):
    bf16 = jnp.bfloat16
    f32 = jnp.float32
    nchunk = SK // rows

    def kv_pairs(hh, b):
        out = []
        for cidx in range(nchunk):
            sl = pl.ds(cidx * rows, rows)
            out.append((pltpu.make_async_copy(k_hbm.at[b, hh, sl], kbuf.at[b, sl], ksem.at[b]),
                        pltpu.make_async_copy(v_hbm.at[b, hh, sl], vbuf.at[b, sl], vsem.at[b])))
        return out

    def start_pairs(pairs):
        for kc, vc in pairs:
            kc.start(priority=0)
            vc.start(priority=1)

    small = [
        pltpu.make_async_copy(x_hbm, x_s, wsem.at[0]),
        pltpu.make_async_copy(c_hbm, c_s, wsem.at[1]),
        pltpu.make_async_copy(wm_hbm, wm_s, wsem.at[2]),
        pltpu.make_async_copy(wq_hbm, wq_s, wsem.at[3]),
    ]
    late = [
        pltpu.make_async_copy(wo_hbm, wo_s, wsem.at[4]),
        pltpu.make_async_copy(wr_hbm, wr_s, wsem.at[5]),
        pltpu.make_async_copy(wg_hbm, wg_s, wsem.at[6]),
        pltpu.make_async_copy(wu_hbm, wu_s, wsem.at[7]),
        pltpu.make_async_copy(wd_hbm, wd_s, wsem.at[8]),
    ]
    small[0].start(priority=0)
    small[1].start(priority=1)
    small[2].start(priority=1)
    small[3].start(priority=0)
    late[0].start(priority=1)
    late[1].start(priority=1)
    late[2].start(priority=0)
    late[3].start(priority=0)
    late[4].start(priority=1)
    if not nodma:
        start_pairs(kv_pairs(0, 0))

    small[0].wait()
    small[1].wait()
    small[2].wait()
    x = x_s[...].astype(f32)
    cc = _silu(c_s[...].astype(f32)).astype(bf16)
    mod = _dot(cc, wm_s[...])
    mod_s[...] = mod
    sa = mod[:, 0 * D:1 * D]
    ca = mod[:, 1 * D:2 * D]
    h = (_layernorm(x) * (1.0 + ca) + sa).astype(bf16)
    if not nodma:
        start_pairs(kv_pairs(0, 1))
    small[3].wait()
    q = _dot(h, wq_s[...])
    q = q * (DH ** -0.5)
    for hh in range(HQ):
        q_s[hh] = q[:, hh * DH:(hh + 1) * DH].astype(bf16)
    if not nodma:
        for b in range(2, dist):
            start_pairs(kv_pairs(0, b))
    else:
        for b in range(B):
            kbuf[b] = jnp.zeros((SK, DH), bf16)
            vbuf[b] = jnp.zeros((SK, DH), bf16)

    late[0].wait()
    row = jax.lax.broadcasted_iota(jnp.int32, (B, DH), 0)
    pk = SK // npiece

    def step(hh, b, oh, prefetch):
        if prefetch and not nodma:
            nb = (b + dist) % B
            pairs = kv_pairs(hh + (b + dist) // B, nb)
        else:
            pairs = []
        grp = len(pairs) // (2 * npiece)
        qh = q_s[hh]
        if not nodma:
            pltpu.make_async_copy(k_hbm.at[0, 0], kbuf.at[b], ksem.at[b]).wait()
        ss = []
        for p in range(npiece):
            ss.append(_dot_nt(qh, kbuf[b, pl.ds(p * pk, pk), :]))
            start_pairs(pairs[p * grp:(p + 1) * grp])
        m = ss[0].max(axis=-1, keepdims=True)
        for s in ss[1:]:
            m = jnp.maximum(m, s.max(axis=-1, keepdims=True))
        if not nodma:
            pltpu.make_async_copy(v_hbm.at[0, 0], vbuf.at[b], vsem.at[b]).wait()
        l = jnp.zeros((B, 1), f32)
        o = jnp.zeros((B, DH), f32)
        for p in range(npiece):
            e = jnp.exp(ss[p] - m)
            l = l + jnp.sum(e, axis=-1, keepdims=True)
            o = o + _dot(e.astype(bf16), vbuf[b, pl.ds(p * pk, pk), :])
            start_pairs(pairs[(npiece + p) * grp:(npiece + p + 1) * grp])
        o = o / l
        return jnp.where(row == b, o, oh)

    def head(hh, acc, last):
        oh = jnp.zeros((B, DH), f32)
        for b in range(B):
            oh = step(hh, b, oh, prefetch=(not last) or (b + dist < B))
        wo_h = wo_s[pl.ds(pl.multiple_of(hh * DH, DH), DH), :]
        return acc + _dot(oh.astype(bf16), wo_h)

    attn = jax.lax.fori_loop(0, HQ - 1, lambda hh, acc: head(hh, acc, False), jnp.zeros((B, D), f32))
    attn = head(HQ - 1, attn, True)

    for cp in late[1:]:
        cp.wait()
    mod = mod_s[...]
    ga = mod[:, 2 * D:3 * D]
    sb = mod[:, 3 * D:4 * D]
    cb = mod[:, 4 * D:5 * D]
    gb = mod[:, 5 * D:6 * D]
    x1 = x_s[...].astype(f32) + ga * attn
    h2 = _layernorm(x1) * (1.0 + cb) + sb
    h2b = h2.astype(bf16)
    wr = wr_s[...].astype(f32)
    h2f = h2b.astype(f32)
    rp = h2f[:, 0:128] * wr[0:1, :]
    for j in range(1, D // 128):
        rp = rp + h2f[:, j * 128:(j + 1) * 128] * wr[j:j + 1, :]
    r = jnp.sum(rp, axis=-1, keepdims=True)
    g = _silu(_dot_nt(h2b, wg_s[...]))
    u = _dot_nt(h2b, wu_s[...])
    y = _dot((g * u).astype(bf16), wd_s[...])
    y = y * jax.nn.sigmoid(r)
    out_ref[...] = (x1 + gb * (h2 + y)).astype(out_ref.dtype)


def _build(dist=3, rows=128, npiece=1, nodma=False):
    bf16 = jnp.bfloat16
    hbm = pl.BlockSpec(memory_space=pltpu.HBM)
    scratch = [
        pltpu.VMEM((B, SK, DH), bf16),
        pltpu.VMEM((B, SK, DH), bf16),
        pltpu.VMEM((B, D), bf16),
        pltpu.VMEM((B, D), bf16),
        pltpu.VMEM((D // 128, 128), bf16),
        pltpu.VMEM((D, HQ * DH), bf16),
        pltpu.VMEM((HQ * DH, D), bf16),
        pltpu.VMEM((FF, D), bf16),
        pltpu.VMEM((FF, D), bf16),
        pltpu.VMEM((FF, D), bf16),
        pltpu.VMEM((D, 6 * D), bf16),
        pltpu.VMEM((HQ, B, DH), bf16),
        pltpu.VMEM((B, 6 * D), jnp.float32),
        pltpu.SemaphoreType.DMA((B,)),
        pltpu.SemaphoreType.DMA((B,)),
        pltpu.SemaphoreType.DMA((9,)),
    ]
    return pl.pallas_call(
        functools.partial(_kernel, dist=dist, rows=rows, npiece=npiece, nodma=nodma),
        out_shape=jax.ShapeDtypeStruct((B, D), bf16),
        in_specs=[hbm] * 11,
        out_specs=pl.BlockSpec(memory_space=pltpu.VMEM),
        scratch_shapes=scratch,
        compiler_params=pltpu.CompilerParams(vmem_limit_bytes=100 * 1024 * 1024),
    )


def _run(A_x, A_k_cache, A_v_cache, A_wq, A_wo, B_x, B_w_r, B_w_gate, B_w_up, B_w_down, c, w_mod, **kw):
    out = _build(**kw)(A_x.reshape(B, D), A_k_cache, A_v_cache, A_wq, A_wo, B_w_r.reshape(D // 128, 128),
                       B_w_gate.T, B_w_up.T, B_w_down, c, w_mod)
    return out.reshape(B, 1, D)


@jax.jit
def pallas_adaLN_cond__gqa_block_cached__moe_arch_mod__decode_kernel(
    A_x: jax.Array,
    A_k_cache: jax.Array,
    A_v_cache: jax.Array,
    A_wq: jax.Array,
    A_wo: jax.Array,
    B_x: jax.Array,
    B_w_r: jax.Array,
    B_w_gate: jax.Array,
    B_w_up: jax.Array,
    B_w_down: jax.Array,
    c: jax.Array,
    w_mod: jax.Array,
):
    return _run(A_x, A_k_cache, A_v_cache, A_wq, A_wo, B_x, B_w_r, B_w_gate, B_w_up, B_w_down, c, w_mod)
```

```python
import functools

import jax
import jax.numpy as jnp
import jax.experimental.pallas as pl
import jax.experimental.pallas.tpu as pltpu

B, D, HQ, SK, DH, FF = 4, 512, 32, 8192, 128, 1376
NSTEP = B * HQ
EPS = 1e-5


def _layernorm(x):
    m = jnp.mean(x, axis=-1, keepdims=True)
    d = x - m
    v = jnp.mean(d * d, axis=-1, keepdims=True)
    return d * jax.lax.rsqrt(v + EPS)


def _silu(x):
    return x * jax.nn.sigmoid(x)


def _dot(a, b):
    return jnp.dot(a, b, preferred_element_type=jnp.float32)


def _dot_nt(a, b):
    return jax.lax.dot_general(a, b, (((1,), (1,)), ((), ())), preferred_element_type=jnp.float32)


def _kernel(x_hbm, k_hbm, v_hbm, wq_hbm, wo_hbm, wr_hbm, wg_hbm, wu_hbm, wd_hbm, c_hbm, wm_hbm,
            out_ref,
            kbuf, vbuf, x_s, c_s, wr_s, wq_s, wo_s, wg_s, wu_s, wd_s, wm_s,
            q_s, mod_s, ksem, vsem, wsem, *, dist, rows, npiece, nodma):
    bf16 = jnp.bfloat16
    f32 = jnp.float32
    nsub = k_hbm.shape[2]
    sub = SK // nsub

    def kv_pairs(hh, b):
        out = []
        for cidx in range(sub // rows):
            sl = pl.ds(cidx * rows, rows)
            out.append((pltpu.make_async_copy(k_hbm.at[b, hh, :, sl], kbuf.at[b, :, sl], ksem.at[b]),
                        pltpu.make_async_copy(v_hbm.at[b, hh, :, sl], vbuf.at[b, :, sl], vsem.at[b])))
        return out

    def start_pairs(pairs):
        for kc, vc in pairs:
            kc.start(priority=0)
            vc.start(priority=1)

    small = [
        pltpu.make_async_copy(x_hbm, x_s, wsem.at[0]),
        pltpu.make_async_copy(c_hbm, c_s, wsem.at[1]),
        pltpu.make_async_copy(wm_hbm, wm_s, wsem.at[2]),
        pltpu.make_async_copy(wq_hbm, wq_s, wsem.at[3]),
    ]
    late = [
        pltpu.make_async_copy(wo_hbm, wo_s, wsem.at[4]),
        pltpu.make_async_copy(wr_hbm, wr_s, wsem.at[5]),
        pltpu.make_async_copy(wg_hbm, wg_s, wsem.at[6]),
        pltpu.make_async_copy(wu_hbm, wu_s, wsem.at[7]),
        pltpu.make_async_copy(wd_hbm, wd_s, wsem.at[8]),
    ]
    small[0].start(priority=0)
    small[1].start(priority=1)
    small[2].start(priority=1)
    small[3].start(priority=0)
    late[0].start(priority=1)
    late[1].start(priority=1)
    late[2].start(priority=0)
    late[3].start(priority=0)
    late[4].start(priority=1)
    if not nodma:
        start_pairs(kv_pairs(0, 0))

    small[0].wait()
    small[1].wait()
    small[2].wait()
    x = x_s[...].astype(f32)
    cc = _silu(c_s[...].astype(f32)).astype(bf16)
    mod = _dot(cc, wm_s[...])
    mod_s[...] = mod
    sa = mod[:, 0 * D:1 * D]
    ca = mod[:, 1 * D:2 * D]
    h = (_layernorm(x) * (1.0 + ca) + sa).astype(bf16)
    if not nodma:
        start_pairs(kv_pairs(0, 1))
    small[3].wait()
    q = _dot(h, wq_s[...])
    q = q * (DH ** -0.5)
    for hh in range(HQ):
        q_s[hh] = q[:, hh * DH:(hh + 1) * DH].astype(bf16)
    if not nodma:
        for b in range(2, dist):
            start_pairs(kv_pairs(0, b))
    else:
        for b in range(B):
            kbuf[b] = jnp.zeros((nsub, sub, DH), bf16)
            vbuf[b] = jnp.zeros((nsub, sub, DH), bf16)

    late[0].wait()
    row = jax.lax.broadcasted_iota(jnp.int32, (B, DH), 0)
    assert npiece == 1

    def step(hh, b, oh, prefetch):
        if prefetch and not nodma:
            nb = (b + dist) % B
            pairs = kv_pairs(hh + (b + dist) // B, nb)
        else:
            pairs = []
        grp = len(pairs) // (2 * npiece)
        qh = q_s[hh]
        if not nodma:
            pltpu.make_async_copy(k_hbm.at[0, 0], kbuf.at[b], ksem.at[b]).wait()
        ss = [_dot_nt(qh, kbuf[b, u]) for u in range(nsub)]
        start_pairs(pairs[:grp])
        m = ss[0].max(axis=-1, keepdims=True)
        for s in ss[1:]:
            m = jnp.maximum(m, s.max(axis=-1, keepdims=True))
        if not nodma:
            pltpu.make_async_copy(v_hbm.at[0, 0], vbuf.at[b], vsem.at[b]).wait()
        l = jnp.zeros((B, 1), f32)
        o = jnp.zeros((B, DH), f32)
        for u in range(nsub):
            e = jnp.exp(ss[u] - m)
            l = l + jnp.sum(e, axis=-1, keepdims=True)
            o = o + _dot(e.astype(bf16), vbuf[b, u])
        start_pairs(pairs[grp:])
        o = o / l
        return jnp.where(row == b, o, oh)

    def head(hh, acc, last):
        oh = jnp.zeros((B, DH), f32)
        for b in range(B):
            oh = step(hh, b, oh, prefetch=(not last) or (b + dist < B))
        wo_h = wo_s[pl.ds(pl.multiple_of(hh * DH, DH), DH), :]
        return acc + _dot(oh.astype(bf16), wo_h)

    attn = jax.lax.fori_loop(0, HQ - 1, lambda hh, acc: head(hh, acc, False), jnp.zeros((B, D), f32))
    attn = head(HQ - 1, attn, True)

    for cp in late[1:]:
        cp.wait()
    mod = mod_s[...]
    ga = mod[:, 2 * D:3 * D]
    sb = mod[:, 3 * D:4 * D]
    cb = mod[:, 4 * D:5 * D]
    gb = mod[:, 5 * D:6 * D]
    x1 = x_s[...].astype(f32) + ga * attn
    h2 = _layernorm(x1) * (1.0 + cb) + sb
    h2b = h2.astype(bf16)
    wr = wr_s[...].astype(f32)
    h2f = h2b.astype(f32)
    rp = h2f[:, 0:128] * wr[0:1, :]
    for j in range(1, D // 128):
        rp = rp + h2f[:, j * 128:(j + 1) * 128] * wr[j:j + 1, :]
    r = jnp.sum(rp, axis=-1, keepdims=True)
    g = _silu(_dot_nt(h2b, wg_s[...]))
    u = _dot_nt(h2b, wu_s[...])
    y = _dot((g * u).astype(bf16), wd_s[...])
    y = y * jax.nn.sigmoid(r)
    out_ref[...] = (x1 + gb * (h2 + y)).astype(out_ref.dtype)


def _build(dist=3, rows=32, npiece=1, nodma=False, nsub=4):
    bf16 = jnp.bfloat16
    hbm = pl.BlockSpec(memory_space=pltpu.HBM)
    scratch = [
        pltpu.VMEM((B, nsub, SK // nsub, DH), bf16),
        pltpu.VMEM((B, nsub, SK // nsub, DH), bf16),
        pltpu.VMEM((B, D), bf16),
        pltpu.VMEM((B, D), bf16),
        pltpu.VMEM((D // 128, 128), bf16),
        pltpu.VMEM((D, HQ * DH), bf16),
        pltpu.VMEM((HQ * DH, D), bf16),
        pltpu.VMEM((FF, D), bf16),
        pltpu.VMEM((FF, D), bf16),
        pltpu.VMEM((FF, D), bf16),
        pltpu.VMEM((D, 6 * D), bf16),
        pltpu.VMEM((HQ, B, DH), bf16),
        pltpu.VMEM((B, 6 * D), jnp.float32),
        pltpu.SemaphoreType.DMA((B,)),
        pltpu.SemaphoreType.DMA((B,)),
        pltpu.SemaphoreType.DMA((9,)),
    ]
    return pl.pallas_call(
        functools.partial(_kernel, dist=dist, rows=rows, npiece=npiece, nodma=nodma),
        out_shape=jax.ShapeDtypeStruct((B, D), bf16),
        in_specs=[hbm] * 11,
        out_specs=pl.BlockSpec(memory_space=pltpu.VMEM),
        scratch_shapes=scratch,
        compiler_params=pltpu.CompilerParams(vmem_limit_bytes=100 * 1024 * 1024),
    )


def _run(A_x, A_k_cache, A_v_cache, A_wq, A_wo, B_x, B_w_r, B_w_gate, B_w_up, B_w_down, c, w_mod, **kw):
    nsub = kw.get('nsub', 4)
    kv_shape = (B, HQ, nsub, SK // nsub, DH)
    out = _build(**kw)(A_x.reshape(B, D), A_k_cache.reshape(kv_shape), A_v_cache.reshape(kv_shape), A_wq, A_wo, B_w_r.reshape(D // 128, 128),
                       B_w_gate.T, B_w_up.T, B_w_down, c, w_mod)
    return out.reshape(B, 1, D)


@jax.jit
def pallas_adaLN_cond__gqa_block_cached__moe_arch_mod__decode_kernel(
    A_x: jax.Array,
    A_k_cache: jax.Array,
    A_v_cache: jax.Array,
    A_wq: jax.Array,
    A_wo: jax.Array,
    B_x: jax.Array,
    B_w_r: jax.Array,
    B_w_gate: jax.Array,
    B_w_up: jax.Array,
    B_w_down: jax.Array,
    c: jax.Array,
    w_mod: jax.Array,
):
    return _run(A_x, A_k_cache, A_v_cache, A_wq, A_wo, B_x, B_w_r, B_w_gate, B_w_up, B_w_down, c, w_mod)
```

```python
import functools

import jax
import jax.numpy as jnp
import jax.experimental.pallas as pl
import jax.experimental.pallas.tpu as pltpu

B, D, HQ, SK, DH, FF = 4, 512, 32, 8192, 128, 1376
EPS = 1e-5

NPIECE = 2
HSTRIDE = 8
NROT = 4
G = NPIECE * NROT
R = SK // G
NSUB = SK // R
NGRP = B * HQ // G
GPB = HQ // G
ROWS = 64
NSLOT = 4
DIST = 3


def _group_head(gg, j):
    i, u = divmod(j, NROT)
    per = HSTRIDE // NROT
    return (gg // per) * (NPIECE * HSTRIDE) + (gg % per) * NROT + i * HSTRIDE + u


def _layernorm(x):
    m = jnp.mean(x, axis=-1, keepdims=True)
    d = x - m
    v = jnp.mean(d * d, axis=-1, keepdims=True)
    return d * jax.lax.rsqrt(v + EPS)


def _silu(x):
    return x * jax.nn.sigmoid(x)


def _dot(a, b):
    return jnp.dot(a, b, preferred_element_type=jnp.float32)


def _dot_nt(a, b):
    return jax.lax.dot_general(a, b, (((1,), (1,)), ((), ())), preferred_element_type=jnp.float32)


def _kernel(x_hbm, k_hbm, v_hbm, wq_hbm, wo_hbm, wr_hbm, wg_hbm, wu_hbm, wd_hbm, c_hbm, wm_hbm,
            out_ref,
            kbuf, vbuf, x_s, c_s, wr_s, wq_s, wo_s, wg_s, wu_s, wd_s, wm_s,
            q_s, mod_s, ksem, vsem, wsem, *, nodma, dist, vrot):
    bf16 = jnp.bfloat16
    f32 = jnp.float32
    per = HSTRIDE // NROT

    def kv_pairs(g, sub):
        slot = sub % NSLOT
        p, q0 = g // per, (g % per) * NROT
        out = []
        for c0 in range(0, R, ROWS):
            src = pl.ds(sub * R + c0, ROWS)
            dst = pl.ds(c0, ROWS)
            for u in range(NROT):
                uv = (u + vrot) % NROT
                out.append((
                    pltpu.make_async_copy(k_hbm.at[p, :, q0 + u, src], kbuf.at[slot, :, u, dst], ksem.at[slot]),
                    pltpu.make_async_copy(v_hbm.at[p, :, q0 + uv, src], vbuf.at[slot, :, uv, dst], vsem.at[slot])))
        return out

    def start_pairs(pairs):
        for kc, vc in pairs:
            kc.start(priority=0)
            vc.start(priority=1)

    small = [
        pltpu.make_async_copy(x_hbm, x_s, wsem.at[0]),
        pltpu.make_async_copy(c_hbm, c_s, wsem.at[1]),
        pltpu.make_async_copy(wm_hbm, wm_s, wsem.at[2]),
        pltpu.make_async_copy(wq_hbm, wq_s, wsem.at[3]),
    ]
    late = [
        pltpu.make_async_copy(wo_hbm, wo_s, wsem.at[4]),
        pltpu.make_async_copy(wr_hbm, wr_s, wsem.at[5]),
        pltpu.make_async_copy(wg_hbm, wg_s, wsem.at[6]),
        pltpu.make_async_copy(wu_hbm, wu_s, wsem.at[7]),
        pltpu.make_async_copy(wd_hbm, wd_s, wsem.at[8]),
    ]
    small[0].start(priority=0)
    small[1].start(priority=1)
    small[2].start(priority=1)
    small[3].start(priority=0)
    late[0].start(priority=1)
    late[1].start(priority=1)
    late[2].start(priority=0)
    late[3].start(priority=0)
    late[4].start(priority=1)
    if not nodma:
        start_pairs(kv_pairs(0, 0))

    small[0].wait()
    small[1].wait()
    small[2].wait()
    x = x_s[...].astype(f32)
    cc = _silu(c_s[...].astype(f32)).astype(bf16)
    mod = _dot(cc, wm_s[...])
    mod_s[...] = mod
    sa = mod[:, 0 * D:1 * D]
    ca = mod[:, 1 * D:2 * D]
    h = (_layernorm(x) * (1.0 + ca) + sa).astype(bf16)
    if not nodma:
        start_pairs(kv_pairs(0, 1))
    small[3].wait()
    q = _dot(h, wq_s[...]) * (DH ** -0.5)
    for b in range(B):
        for gg in range(GPB):
            for j in range(G):
                hd = _group_head(gg, j)
                q_s[b * GPB + gg, j:j + 1, :] = q[b:b + 1, hd * DH:(hd + 1) * DH]
    if not nodma:
        for s in range(2, dist):
            start_pairs(kv_pairs(0, s))
    else:
        for s in range(NSLOT):
            kbuf[s] = jnp.zeros(kbuf.shape[1:], bf16)
            vbuf[s] = jnp.zeros(vbuf.shape[1:], bf16)

    late[0].wait()
    row_s = jax.lax.broadcasted_iota(jnp.int32, (G, R), 0)
    row_o = jax.lax.broadcasted_iota(jnp.int32, (G, DH), 0)
    row_a = jax.lax.broadcasted_iota(jnp.int32, (G, D), 0)
    row_b = jax.lax.broadcasted_iota(jnp.int32, (B, D), 0)

    def substep(g, sub, qg, state, pairs):
        slot = sub % NSLOT
        half = len(pairs) // 2
        if not nodma:
            pltpu.make_async_copy(kbuf.at[slot], kbuf.at[slot], ksem.at[slot]).wait()
        s = None
        for j in range(G):
            sj = _dot_nt(qg, kbuf[slot, j // NROT, j % NROT])
            s = sj if s is None else jnp.where(row_s == j, sj, s)
        start_pairs(pairs[:half])
        mcur = jnp.max(s, axis=-1, keepdims=True)
        if state is None:
            m = mcur
        else:
            m_old, l_old, o_old = state
            m = jnp.maximum(m_old, mcur)
        e = jnp.exp(s - m)
        l = jnp.sum(e, axis=-1, keepdims=True)
        eb = e.astype(bf16)
        if not nodma:
            pltpu.make_async_copy(vbuf.at[slot], vbuf.at[slot], vsem.at[slot]).wait()
        o = None
        for j in range(G):
            oj = _dot(eb, vbuf[slot, j // NROT, j % NROT])
            o = oj if o is None else jnp.where(row_o == j, oj, o)
        start_pairs(pairs[half:])
        if state is not None:
            alpha = jnp.exp(m_old - m)
            l = l + alpha * l_old
            o = o + alpha * o_old
        return m, l, o

    def group(g, attn, last):
        qg = q_s[g].astype(bf16)
        state = None
        for sub in range(NSUB):
            nxt = sub + dist
            if nodma or (last and nxt >= NSUB):
                pairs = []
            else:
                pairs = kv_pairs(g + nxt // NSUB, nxt % NSUB)
            state = substep(g, sub, qg, state, pairs)
        _, l, o = state
        ob = (o / l).astype(bf16)
        gg = g % GPB
        h0 = (gg // per) * (NPIECE * HSTRIDE) + (gg % per) * NROT
        t = None
        for j in range(G):
            tj = _dot(ob, wo_s[h0 + (j // NROT) * HSTRIDE + j % NROT])
            t = tj if t is None else jnp.where(row_a == j, tj, t)
        tsum = jnp.sum(t, axis=0, keepdims=True)
        return attn + jnp.where(row_b == g // GPB, tsum, 0.0)

    attn = jax.lax.fori_loop(0, NGRP - 1, lambda g, a: group(g, a, False), jnp.zeros((B, D), f32))
    attn = group(NGRP - 1, attn, True)

    for cp in late[1:]:
        cp.wait()
    mod = mod_s[...]
    ga = mod[:, 2 * D:3 * D]
    sb = mod[:, 3 * D:4 * D]
    cb = mod[:, 4 * D:5 * D]
    gb = mod[:, 5 * D:6 * D]
    x1 = x_s[...].astype(f32) + ga * attn
    h2 = _layernorm(x1) * (1.0 + cb) + sb
    h2b = h2.astype(bf16)
    wr = wr_s[...].astype(f32)
    h2f = h2b.astype(f32)
    rp = h2f[:, 0:128] * wr[0:1, :]
    for j in range(1, D // 128):
        rp = rp + h2f[:, j * 128:(j + 1) * 128] * wr[j:j + 1, :]
    r = jnp.sum(rp, axis=-1, keepdims=True)
    g = _silu(_dot_nt(h2b, wg_s[...]))
    u = _dot_nt(h2b, wu_s[...])
    y = _dot((g * u).astype(bf16), wd_s[...])
    y = y * jax.nn.sigmoid(r)
    out_ref[...] = (x1 + gb * (h2 + y)).astype(out_ref.dtype)


def _build(nodma=False, dist=DIST, vrot=0):
    bf16 = jnp.bfloat16
    hbm = pl.BlockSpec(memory_space=pltpu.HBM)
    scratch = [
        pltpu.VMEM((NSLOT, NPIECE, NROT, R, DH), bf16),
        pltpu.VMEM((NSLOT, NPIECE, NROT, R, DH), bf16),
        pltpu.VMEM((B, D), bf16),
        pltpu.VMEM((B, D), bf16),
        pltpu.VMEM((D // 128, 128), bf16),
        pltpu.VMEM((D, HQ * DH), bf16),
        pltpu.VMEM((HQ, DH, D), bf16),
        pltpu.VMEM((FF, D), bf16),
        pltpu.VMEM((FF, D), bf16),
        pltpu.VMEM((FF, D), bf16),
        pltpu.VMEM((D, 6 * D), bf16),
        pltpu.VMEM((NGRP, G, DH), jnp.float32),
        pltpu.VMEM((B, 6 * D), jnp.float32),
        pltpu.SemaphoreType.DMA((NSLOT,)),
        pltpu.SemaphoreType.DMA((NSLOT,)),
        pltpu.SemaphoreType.DMA((9,)),
    ]
    return pl.pallas_call(
        functools.partial(_kernel, nodma=nodma, dist=dist, vrot=vrot),
        out_shape=jax.ShapeDtypeStruct((B, D), bf16),
        in_specs=[hbm] * 11,
        out_specs=pl.BlockSpec(memory_space=pltpu.VMEM),
        scratch_shapes=scratch,
        compiler_params=pltpu.CompilerParams(vmem_limit_bytes=100 * 1024 * 1024),
    )


def _run(A_x, A_k_cache, A_v_cache, A_wq, A_wo, B_x, B_w_r, B_w_gate, B_w_up, B_w_down, c, w_mod, **kw):
    kv_shape = (B * HQ // (NPIECE * HSTRIDE), NPIECE, HSTRIDE, SK, DH)
    out = _build(**kw)(A_x.reshape(B, D), A_k_cache.reshape(kv_shape), A_v_cache.reshape(kv_shape),
                       A_wq, A_wo.reshape(HQ, DH, D), B_w_r.reshape(D // 128, 128),
                       B_w_gate.T, B_w_up.T, B_w_down, c, w_mod)
    return out.reshape(B, 1, D)


@jax.jit
def pallas_adaLN_cond__gqa_block_cached__moe_arch_mod__decode_kernel(
    A_x: jax.Array,
    A_k_cache: jax.Array,
    A_v_cache: jax.Array,
    A_wq: jax.Array,
    A_wo: jax.Array,
    B_x: jax.Array,
    B_w_r: jax.Array,
    B_w_gate: jax.Array,
    B_w_up: jax.Array,
    B_w_down: jax.Array,
    c: jax.Array,
    w_mod: jax.Array,
):
    return _run(A_x, A_k_cache, A_v_cache, A_wq, A_wo, B_x, B_w_r, B_w_gate, B_w_up, B_w_down, c, w_mod)
```

```python
import functools

import jax
import jax.numpy as jnp
import jax.experimental.pallas as pl
import jax.experimental.pallas.tpu as pltpu

B, D, HQ, SK, DH, FF = 4, 512, 32, 8192, 128, 1376
EPS = 1e-5

NPIECE = 2
HSTRIDE = 8
NROT = 4
G = NPIECE * NROT
R = SK // G
NSUB = SK // R
NGRP = B * HQ // G
GPB = HQ // G
ROWS = 64
NSLOT = 4
DIST = 2


def _group_head(gg, j):
    i, u = divmod(j, NROT)
    per = HSTRIDE // NROT
    return (gg // per) * (NPIECE * HSTRIDE) + (gg % per) * NROT + i * HSTRIDE + u


def _layernorm(x):
    m = jnp.mean(x, axis=-1, keepdims=True)
    d = x - m
    v = jnp.mean(d * d, axis=-1, keepdims=True)
    return d * jax.lax.rsqrt(v + EPS)


def _silu(x):
    return x * jax.nn.sigmoid(x)


def _dot(a, b):
    return jnp.dot(a, b, preferred_element_type=jnp.float32)


def _dot_nt(a, b):
    return jax.lax.dot_general(a, b, (((1,), (1,)), ((), ())), preferred_element_type=jnp.float32)


def _kernel(x_hbm, k_hbm, v_hbm, wq_hbm, wo_hbm, wr_hbm, wg_hbm, wu_hbm, wd_hbm, c_hbm, wm_hbm,
            out_ref,
            kbuf, vbuf, x_s, c_s, wr_s, wq_s, wo_s, wg_s, wu_s, wd_s, wm_s,
            q_s, mod_s, ksem, vsem, wsem, msem, *, dist, vrot, tail, fchunks):
    bf16 = jnp.bfloat16
    f32 = jnp.float32
    per = HSTRIDE // NROT

    def kv_pairs(g, sub):
        slot = sub % NSLOT
        p, q0 = g // per, (g % per) * NROT
        out = []
        for c0 in range(0, R, ROWS):
            src = pl.ds(sub * R + c0, ROWS)
            dst = pl.ds(c0, ROWS)
            for u in range(NROT):
                uv = (u + vrot) % NROT
                out.append((
                    pltpu.make_async_copy(k_hbm.at[p, :, q0 + u, src], kbuf.at[slot, :, u, dst], ksem.at[slot]),
                    pltpu.make_async_copy(v_hbm.at[p, :, q0 + uv, src], vbuf.at[slot, :, uv, dst], vsem.at[slot])))
        return out

    def start_pairs(pairs):
        for kc, vc in pairs:
            kc.start(priority=0)
            if vc is not None:
                vc.start(priority=1)

    def tile_copies(src, dst, sem, rows, cols=None):
        n, w = dst.shape
        cols = cols or w
        return [pltpu.make_async_copy(src.at[pl.ds(r, min(rows, n - r)), pl.ds(c0, cols)],
                                      dst.at[pl.ds(r, min(rows, n - r)), pl.ds(c0, cols)], sem)
                for r in range(0, n, rows) for c0 in range(0, w, cols)]

    def wait_all(buf, sem):
        pltpu.make_async_copy(buf, buf, sem).wait()

    wq_cp = tile_copies(wq_hbm, wq_s, wsem.at[2], 16, 1024)
    wm_cp = tile_copies(wm_hbm, wm_s, wsem.at[3], 16, 1024)
    wo_cp = tile_copies(wo_hbm, wo_s, wsem.at[4], 32)
    n_a = len(wq_cp) - len(wm_cp)
    head_a = list(zip(wq_cp, wm_cp + wo_cp[:n_a]))
    rest = wo_cp[n_a:]
    head_b = list(zip(rest[:len(rest) // 2], rest[len(rest) // 2:]))
    mlp_pairs = []
    slab_end = []
    for f, (f0, fn) in enumerate(fchunks):
        sl = pl.ds(f0, fn)
        cps = [tile_copies(src.at[sl], dst.at[sl], msem.at[f, t], 32)
               for t, (src, dst) in enumerate(((wg_hbm, wg_s), (wu_hbm, wu_s), (wd_hbm, wd_s)))]
        d = cps[2]
        dh = (len(d) + 1) // 2
        mlp_pairs += list(zip(cps[0] + d[:dh], cps[1] + d[dh:] + [None] * (2 * dh - len(d))))
        slab_end.append(len(mlp_pairs))
    n_mlp = len(mlp_pairs)


    def take_mlp(n):
        out = mlp_pairs[:n]
        del mlp_pairs[:n]
        return out

    x_cp = pltpu.make_async_copy(x_hbm, x_s, wsem.at[0])
    c_cp = pltpu.make_async_copy(c_hbm, c_s, wsem.at[1])
    wr_cp = pltpu.make_async_copy(wr_hbm, wr_s, wsem.at[5])
    x_cp.start(priority=0)
    c_cp.start(priority=1)
    wr_cp.start(priority=1)
    start_pairs(head_a)
    start_pairs(head_b)

    x_cp.wait()
    c_cp.wait()
    wait_all(wm_s, wsem.at[3])
    x = x_s[...].astype(f32)
    cc = _silu(c_s[...].astype(f32)).astype(bf16)
    mod = _dot(cc, wm_s[...])
    mod_s[...] = mod
    sa = mod[:, 0 * D:1 * D]
    ca = mod[:, 1 * D:2 * D]
    h = (_layernorm(x) * (1.0 + ca) + sa).astype(bf16)
    kv0 = kv_pairs(0, 0)
    start_pairs(kv0[:len(kv0) // 2])
    wait_all(wq_s, wsem.at[2])
    q = _dot(h, wq_s[...]) * (DH ** -0.5)
    start_pairs(kv0[len(kv0) // 2:])
    for b in range(B):
        for gg in range(GPB):
            for j in range(G):
                hd = _group_head(gg, j)
                q_s[b * GPB + gg, j:j + 1, :] = q[b:b + 1, hd * DH:(hd + 1) * DH]
    for s in range(1, dist):
        start_pairs(kv_pairs(0, s))

    wait_all(wo_s, wsem.at[4])
    row_s = jax.lax.broadcasted_iota(jnp.int32, (G, R), 0)
    row_o = jax.lax.broadcasted_iota(jnp.int32, (G, DH), 0)
    row_a = jax.lax.broadcasted_iota(jnp.int32, (G, D), 0)
    row_b = jax.lax.broadcasted_iota(jnp.int32, (B, D), 0)

    def substep(g, sub, qg, state, pairs_a, pairs_b):
        slot = sub % NSLOT
        wait_all(kbuf.at[slot], ksem.at[slot])
        s = None
        for j in range(G):
            sj = _dot_nt(qg, kbuf[slot, j // NROT, j % NROT])
            s = sj if s is None else jnp.where(row_s == j, sj, s)
        start_pairs(pairs_a)
        mcur = jnp.max(s, axis=-1, keepdims=True)
        if state is None:
            m = mcur
        else:
            m_old, l_old, o_old = state
            m = jnp.maximum(m_old, mcur)
        e = jnp.exp(s - m)
        l = jnp.sum(e, axis=-1, keepdims=True)
        eb = e.astype(bf16)
        wait_all(vbuf.at[slot], vsem.at[slot])
        o = None
        for j in range(G):
            oj = _dot(eb, vbuf[slot, j // NROT, j % NROT])
            o = oj if o is None else jnp.where(row_o == j, oj, o)
        start_pairs(pairs_b)
        if state is not None:
            alpha = jnp.exp(m_old - m)
            l = l + alpha * l_old
            o = o + alpha * o_old
        return m, l, o

    def group(g, attn, last):
        qg = q_s[g].astype(bf16)
        state = None
        for sub in range(NSUB):
            nxt = sub + dist
            if last and nxt >= NSUB:
                pa = take_mlp(tail[2 * (nxt - NSUB)])
                pb = take_mlp(tail[2 * (nxt - NSUB) + 1])
            else:
                pairs = kv_pairs(g + nxt // NSUB, nxt % NSUB)
                pa, pb = pairs[:len(pairs) // 2], pairs[len(pairs) // 2:]
            state = substep(g, sub, qg, state, pa, pb)
        _, l, o = state
        ob = (o / l).astype(bf16)
        gg = g % GPB
        h0 = (gg // per) * (NPIECE * HSTRIDE) + (gg % per) * NROT
        t = None
        for j in range(G):
            hd = h0 + (j // NROT) * HSTRIDE + j % NROT
            tj = _dot(ob, wo_s[pl.ds(pl.multiple_of(hd * DH, DH), DH), :])
            t = tj if t is None else jnp.where(row_a == j, tj, t)
        tsum = jnp.sum(t, axis=0, keepdims=True)
        return attn + jnp.where(row_b == g // GPB, tsum, 0.0)

    attn = jax.lax.fori_loop(0, NGRP - 1, lambda g, a: group(g, a, False), jnp.zeros((B, D), f32))
    attn = group(NGRP - 1, attn, True)

    start_pairs(take_mlp(tail[2 * dist]))
    wr_cp.wait()
    mod = mod_s[...]
    ga = mod[:, 2 * D:3 * D]
    sb = mod[:, 3 * D:4 * D]
    cb = mod[:, 4 * D:5 * D]
    gb = mod[:, 5 * D:6 * D]
    x1 = x_s[...].astype(f32) + ga * attn
    h2 = _layernorm(x1) * (1.0 + cb) + sb
    h2b = h2.astype(bf16)
    wr = wr_s[...].astype(f32)
    h2f = h2b.astype(f32)
    rp = h2f[:, 0:128] * wr[0:1, :]
    for j in range(1, D // 128):
        rp = rp + h2f[:, j * 128:(j + 1) * 128] * wr[j:j + 1, :]
    gate = gb * jax.nn.sigmoid(jnp.sum(rp, axis=-1, keepdims=True))
    base = x1 + gb * h2
    start_pairs(take_mlp(tail[2 * dist + 1]))
    y = None
    for f, (f0, fn) in enumerate(fchunks):
        sl = pl.ds(f0, fn)
        start_pairs(take_mlp(len(mlp_pairs) if f == len(fchunks) - 1 else tail[-1]))
        assert n_mlp - len(mlp_pairs) >= slab_end[f], "slab awaited before it was issued"
        for t, buf in enumerate((wg_s, wu_s, wd_s)):
            wait_all(buf.at[sl], msem.at[f, t])
        g = _silu(_dot_nt(h2b, wg_s[sl, :]))
        u = _dot_nt(h2b, wu_s[sl, :])
        yf = _dot((g * u).astype(bf16), wd_s[sl, :])
        y = yf if y is None else y + yf
    out_ref[...] = (base + gate * y).astype(out_ref.dtype)


def _build(dist=DIST, vrot=0, tail=(18, 18, 6, 6, 4, 5, 8), fslab=256):
    fchunks = tuple((f0, min(fslab, FF - f0)) for f0 in range(0, FF, fslab))
    bf16 = jnp.bfloat16
    hbm = pl.BlockSpec(memory_space=pltpu.HBM)
    scratch = [
        pltpu.VMEM((NSLOT, NPIECE, NROT, R, DH), bf16),
        pltpu.VMEM((NSLOT, NPIECE, NROT, R, DH), bf16),
        pltpu.VMEM((B, D), bf16),
        pltpu.VMEM((B, D), bf16),
        pltpu.VMEM((D // 128, 128), bf16),
        pltpu.VMEM((D, HQ * DH), bf16),
        pltpu.VMEM((HQ * DH, D), bf16),
        pltpu.VMEM((FF, D), bf16),
        pltpu.VMEM((FF, D), bf16),
        pltpu.VMEM((FF, D), bf16),
        pltpu.VMEM((D, 6 * D), bf16),
        pltpu.VMEM((NGRP, G, DH), jnp.float32),
        pltpu.VMEM((B, 6 * D), jnp.float32),
        pltpu.SemaphoreType.DMA((NSLOT,)),
        pltpu.SemaphoreType.DMA((NSLOT,)),
        pltpu.SemaphoreType.DMA((6,)),
        pltpu.SemaphoreType.DMA((len(fchunks), 3)),
    ]
    return pl.pallas_call(
        functools.partial(_kernel, dist=dist, vrot=vrot, tail=tail, fchunks=fchunks),
        out_shape=jax.ShapeDtypeStruct((B, D), bf16),
        in_specs=[hbm] * 11,
        out_specs=pl.BlockSpec(memory_space=pltpu.VMEM),
        scratch_shapes=scratch,
        compiler_params=pltpu.CompilerParams(vmem_limit_bytes=100 * 1024 * 1024),
    )


def _run(A_x, A_k_cache, A_v_cache, A_wq, A_wo, B_x, B_w_r, B_w_gate, B_w_up, B_w_down, c, w_mod, **kw):
    kv_shape = (B * HQ // (NPIECE * HSTRIDE), NPIECE, HSTRIDE, SK, DH)
    out = _build(**kw)(A_x.reshape(B, D), A_k_cache.reshape(kv_shape), A_v_cache.reshape(kv_shape),
                       A_wq, A_wo, B_w_r.reshape(D // 128, 128),
                       B_w_gate.T, B_w_up.T, B_w_down, c, w_mod)
    return out.reshape(B, 1, D)


@jax.jit
def pallas_adaLN_cond__gqa_block_cached__moe_arch_mod__decode_kernel(
    A_x: jax.Array,
    A_k_cache: jax.Array,
    A_v_cache: jax.Array,
    A_wq: jax.Array,
    A_wo: jax.Array,
    B_x: jax.Array,
    B_w_r: jax.Array,
    B_w_gate: jax.Array,
    B_w_up: jax.Array,
    B_w_down: jax.Array,
    c: jax.Array,
    w_mod: jax.Array,
):
    return _run(A_x, A_k_cache, A_v_cache, A_wq, A_wo, B_x, B_w_r, B_w_gate, B_w_up, B_w_down, c, w_mod)
```

```python
import functools

import jax
import jax.numpy as jnp
import jax.experimental.pallas as pl
import jax.experimental.pallas.tpu as pltpu

B, D, HQ, SK, DH, FF = 4, 512, 32, 8192, 128, 1376
EPS = 1e-5

NPIECE = 2
HSTRIDE = 8
NROT = 4
G = NPIECE * NROT
R = SK // G
NSUB = SK // R
NGRP = B * HQ // G
GPB = HQ // G
ROWS = 64
NSLOT = 4
DIST = 2


def _group_head(gg, j):
    i, u = divmod(j, NROT)
    per = HSTRIDE // NROT
    return (gg // per) * (NPIECE * HSTRIDE) + (gg % per) * NROT + i * HSTRIDE + u


def _layernorm(x):
    m = jnp.mean(x, axis=-1, keepdims=True)
    d = x - m
    v = jnp.mean(d * d, axis=-1, keepdims=True)
    return d * jax.lax.rsqrt(v + EPS)


def _silu(x):
    return x * jax.nn.sigmoid(x)


def _dot(a, b):
    return jnp.dot(a, b, preferred_element_type=jnp.float32)


def _dot_nt(a, b):
    return jax.lax.dot_general(a, b, (((1,), (1,)), ((), ())), preferred_element_type=jnp.float32)


def _kernel(x_hbm, k_hbm, v_hbm, wq_hbm, wo_hbm, wr_hbm, wg_hbm, wu_hbm, wd_hbm, c_hbm, wm_hbm,
            out_ref,
            kbuf, vbuf, x_s, c_s, wr_s, wq_s, wo_s, wg_s, wu_s, wd_s, wm_s,
            q_s, mod_s, ksem, vsem, wsem, msem, *, dist, vrot, tail, fchunks, hrot, mrot):
    bf16 = jnp.bfloat16
    f32 = jnp.float32
    per = HSTRIDE // NROT

    def kv_pairs(g, sub):
        slot = sub % NSLOT
        p, q0 = g // per, (g % per) * NROT
        out = []
        for c0 in range(0, R, ROWS):
            src = pl.ds(sub * R + c0, ROWS)
            dst = pl.ds(c0, ROWS)
            for u in range(NROT):
                uv = (u + vrot) % NROT
                out.append((
                    pltpu.make_async_copy(k_hbm.at[p, :, q0 + u, src], kbuf.at[slot, :, u, dst], ksem.at[slot]),
                    pltpu.make_async_copy(v_hbm.at[p, :, q0 + uv, src], vbuf.at[slot, :, uv, dst], vsem.at[slot])))
        return out

    def start_pairs(pairs):
        for kc, vc in pairs:
            kc.start(priority=0)
            if vc is not None:
                vc.start(priority=1)

    def tile_copies(src, dst, sem, rows, cols=None, rot=1):
        n, w = dst.shape
        cols = cols or w
        span = n // rot
        out = []
        for r in range(0, span, rows):
            for c0 in range(0, w, cols):
                for k in range(rot):
                    idx = (pl.ds(k * span + r, min(rows, span - r)), pl.ds(c0, cols))
                    out.append(pltpu.make_async_copy(src.at[idx], dst.at[idx], sem))
        return out

    def wait_all(buf, sem):
        pltpu.make_async_copy(buf, buf, sem).wait()

    wq_cp = tile_copies(wq_hbm, wq_s, wsem.at[2], 16, 1024, hrot)
    wm_cp = tile_copies(wm_hbm, wm_s, wsem.at[3], 16, 1024, hrot)
    wo_cp = tile_copies(wo_hbm, wo_s, wsem.at[4], 32, None, hrot)
    n_a = len(wq_cp) - len(wm_cp)
    head_a = list(zip(wq_cp, wm_cp + wo_cp[:n_a]))
    rest = wo_cp[n_a:]
    head_b = list(zip(rest[:len(rest) // 2], rest[len(rest) // 2:]))
    mlp_pairs = []
    slab_end = []
    for f, (f0, fn) in enumerate(fchunks):
        sl = pl.ds(f0, fn)
        cps = [tile_copies(src.at[sl], dst.at[sl], msem.at[f, t], 32)
               for t, (src, dst) in enumerate(((wg_hbm, wg_s), (wu_hbm, wu_s), (wd_hbm, wd_s)))]
        if mrot:
            flat = [cp for trio in zip(*cps) for cp in trio]
            mlp_pairs += list(zip(flat[0::2], flat[1::2] + [None] * (len(flat) % 2)))
        else:
            d = cps[2]
            dh = (len(d) + 1) // 2
            mlp_pairs += list(zip(cps[0] + d[:dh], cps[1] + d[dh:] + [None] * (2 * dh - len(d))))
        slab_end.append(len(mlp_pairs))
    n_mlp = len(mlp_pairs)


    def take_mlp(n):
        out = mlp_pairs[:n]
        del mlp_pairs[:n]
        return out

    x_cp = pltpu.make_async_copy(x_hbm, x_s, wsem.at[0])
    c_cp = pltpu.make_async_copy(c_hbm, c_s, wsem.at[1])
    wr_cp = pltpu.make_async_copy(wr_hbm, wr_s, wsem.at[5])
    x_cp.start(priority=0)
    c_cp.start(priority=1)
    wr_cp.start(priority=1)
    start_pairs(head_a)
    start_pairs(head_b)

    x_cp.wait()
    c_cp.wait()
    wait_all(wm_s, wsem.at[3])
    x = x_s[...].astype(f32)
    cc = _silu(c_s[...].astype(f32)).astype(bf16)
    mod = _dot(cc, wm_s[...])
    mod_s[...] = mod
    sa = mod[:, 0 * D:1 * D]
    ca = mod[:, 1 * D:2 * D]
    h = (_layernorm(x) * (1.0 + ca) + sa).astype(bf16)
    kv0 = kv_pairs(0, 0)
    start_pairs(kv0[:len(kv0) // 2])
    wait_all(wq_s, wsem.at[2])
    q = _dot(h, wq_s[...]) * (DH ** -0.5)
    start_pairs(kv0[len(kv0) // 2:])
    for b in range(B):
        for gg in range(GPB):
            for j in range(G):
                hd = _group_head(gg, j)
                q_s[b * GPB + gg, j:j + 1, :] = q[b:b + 1, hd * DH:(hd + 1) * DH]
    for s in range(1, dist):
        start_pairs(kv_pairs(0, s))

    wait_all(wo_s, wsem.at[4])
    row_s = jax.lax.broadcasted_iota(jnp.int32, (G, R), 0)
    row_o = jax.lax.broadcasted_iota(jnp.int32, (G, DH), 0)
    row_a = jax.lax.broadcasted_iota(jnp.int32, (G, D), 0)
    row_b = jax.lax.broadcasted_iota(jnp.int32, (B, D), 0)

    def substep(g, sub, qg, state, pairs_a, pairs_b):
        slot = sub % NSLOT
        wait_all(kbuf.at[slot], ksem.at[slot])
        s = None
        for j in range(G):
            sj = _dot_nt(qg, kbuf[slot, j // NROT, j % NROT])
            s = sj if s is None else jnp.where(row_s == j, sj, s)
        start_pairs(pairs_a)
        mcur = jnp.max(s, axis=-1, keepdims=True)
        if state is None:
            m = mcur
        else:
            m_old, l_old, o_old = state
            m = jnp.maximum(m_old, mcur)
        e = jnp.exp(s - m)
        l = jnp.sum(e, axis=-1, keepdims=True)
        eb = e.astype(bf16)
        wait_all(vbuf.at[slot], vsem.at[slot])
        o = None
        for j in range(G):
            oj = _dot(eb, vbuf[slot, j // NROT, j % NROT])
            o = oj if o is None else jnp.where(row_o == j, oj, o)
        start_pairs(pairs_b)
        if state is not None:
            alpha = jnp.exp(m_old - m)
            l = l + alpha * l_old
            o = o + alpha * o_old
        return m, l, o

    def group(g, attn, last):
        qg = q_s[g].astype(bf16)
        state = None
        for sub in range(NSUB):
            nxt = sub + dist
            if last and nxt >= NSUB:
                pa = take_mlp(tail[2 * (nxt - NSUB)])
                pb = take_mlp(tail[2 * (nxt - NSUB) + 1])
            else:
                pairs = kv_pairs(g + nxt // NSUB, nxt % NSUB)
                pa, pb = pairs[:len(pairs) // 2], pairs[len(pairs) // 2:]
            state = substep(g, sub, qg, state, pa, pb)
        _, l, o = state
        ob = (o / l).astype(bf16)
        gg = g % GPB
        h0 = (gg // per) * (NPIECE * HSTRIDE) + (gg % per) * NROT
        t = None
        for j in range(G):
            hd = h0 + (j // NROT) * HSTRIDE + j % NROT
            tj = _dot(ob, wo_s[pl.ds(pl.multiple_of(hd * DH, DH), DH), :])
            t = tj if t is None else jnp.where(row_a == j, tj, t)
        tsum = jnp.sum(t, axis=0, keepdims=True)
        return attn + jnp.where(row_b == g // GPB, tsum, 0.0)

    attn = jax.lax.fori_loop(0, NGRP - 1, lambda g, a: group(g, a, False), jnp.zeros((B, D), f32))
    attn = group(NGRP - 1, attn, True)

    start_pairs(take_mlp(tail[2 * dist]))
    wr_cp.wait()
    mod = mod_s[...]
    ga = mod[:, 2 * D:3 * D]
    sb = mod[:, 3 * D:4 * D]
    cb = mod[:, 4 * D:5 * D]
    gb = mod[:, 5 * D:6 * D]
    x1 = x_s[...].astype(f32) + ga * attn
    h2 = _layernorm(x1) * (1.0 + cb) + sb
    h2b = h2.astype(bf16)
    wr = wr_s[...].astype(f32)
    h2f = h2b.astype(f32)
    rp = h2f[:, 0:128] * wr[0:1, :]
    for j in range(1, D // 128):
        rp = rp + h2f[:, j * 128:(j + 1) * 128] * wr[j:j + 1, :]
    gate = gb * jax.nn.sigmoid(jnp.sum(rp, axis=-1, keepdims=True))
    base = x1 + gb * h2
    start_pairs(take_mlp(tail[2 * dist + 1]))
    y = None
    for f, (f0, fn) in enumerate(fchunks):
        sl = pl.ds(f0, fn)
        start_pairs(take_mlp(len(mlp_pairs) if f == len(fchunks) - 1 else tail[-1]))
        assert n_mlp - len(mlp_pairs) >= slab_end[f], "slab awaited before it was issued"
        for t, buf in enumerate((wg_s, wu_s, wd_s)):
            wait_all(buf.at[sl], msem.at[f, t])
        g = _silu(_dot_nt(h2b, wg_s[sl, :]))
        u = _dot_nt(h2b, wu_s[sl, :])
        yf = _dot((g * u).astype(bf16), wd_s[sl, :])
        y = yf if y is None else y + yf
    out_ref[...] = (base + gate * y).astype(out_ref.dtype)


def _build(dist=DIST, vrot=0, tail=(18, 18, 6, 6, 4, 5, 8), fslab=256, hrot=4, mrot=True):
    fchunks = tuple((f0, min(fslab, FF - f0)) for f0 in range(0, FF, fslab))
    bf16 = jnp.bfloat16
    hbm = pl.BlockSpec(memory_space=pltpu.HBM)
    scratch = [
        pltpu.VMEM((NSLOT, NPIECE, NROT, R, DH), bf16),
        pltpu.VMEM((NSLOT, NPIECE, NROT, R, DH), bf16),
        pltpu.VMEM((B, D), bf16),
        pltpu.VMEM((B, D), bf16),
        pltpu.VMEM((D // 128, 128), bf16),
        pltpu.VMEM((D, HQ * DH), bf16),
        pltpu.VMEM((HQ * DH, D), bf16),
        pltpu.VMEM((FF, D), bf16),
        pltpu.VMEM((FF, D), bf16),
        pltpu.VMEM((FF, D), bf16),
        pltpu.VMEM((D, 6 * D), bf16),
        pltpu.VMEM((NGRP, G, DH), jnp.float32),
        pltpu.VMEM((B, 6 * D), jnp.float32),
        pltpu.SemaphoreType.DMA((NSLOT,)),
        pltpu.SemaphoreType.DMA((NSLOT,)),
        pltpu.SemaphoreType.DMA((6,)),
        pltpu.SemaphoreType.DMA((len(fchunks), 3)),
    ]
    return pl.pallas_call(
        functools.partial(_kernel, dist=dist, vrot=vrot, tail=tail, fchunks=fchunks, hrot=hrot, mrot=mrot),
        out_shape=jax.ShapeDtypeStruct((B, D), bf16),
        in_specs=[hbm] * 11,
        out_specs=pl.BlockSpec(memory_space=pltpu.VMEM),
        scratch_shapes=scratch,
        compiler_params=pltpu.CompilerParams(vmem_limit_bytes=100 * 1024 * 1024),
    )


def _run(A_x, A_k_cache, A_v_cache, A_wq, A_wo, B_x, B_w_r, B_w_gate, B_w_up, B_w_down, c, w_mod, **kw):
    kv_shape = (B * HQ // (NPIECE * HSTRIDE), NPIECE, HSTRIDE, SK, DH)
    out = _build(**kw)(A_x.reshape(B, D), A_k_cache.reshape(kv_shape), A_v_cache.reshape(kv_shape),
                       A_wq, A_wo, B_w_r.reshape(D // 128, 128),
                       B_w_gate.T, B_w_up.T, B_w_down, c, w_mod)
    return out.reshape(B, 1, D)


@jax.jit
def pallas_adaLN_cond__gqa_block_cached__moe_arch_mod__decode_kernel(
    A_x: jax.Array,
    A_k_cache: jax.Array,
    A_v_cache: jax.Array,
    A_wq: jax.Array,
    A_wo: jax.Array,
    B_x: jax.Array,
    B_w_r: jax.Array,
    B_w_gate: jax.Array,
    B_w_up: jax.Array,
    B_w_down: jax.Array,
    c: jax.Array,
    w_mod: jax.Array,
):
    return _run(A_x, A_k_cache, A_v_cache, A_wq, A_wo, B_x, B_w_r, B_w_gate, B_w_up, B_w_down, c, w_mod)
```

```python
import functools

import jax
import jax.numpy as jnp
import jax.experimental.pallas as pl
import jax.experimental.pallas.tpu as pltpu

B, D, HQ, SK, DH, FF = 4, 512, 32, 8192, 128, 1376
EPS = 1e-5

NPIECE = 2
HSTRIDE = 8
NROT = 4
G = NPIECE * NROT
R = SK // G
NSUB = SK // R
NGRP = B * HQ // G
GPB = HQ // G
ROWS = 64
NSLOT = 4
DIST = 2


def _group_head(gg, j):
    i, u = divmod(j, NROT)
    per = HSTRIDE // NROT
    return (gg // per) * (NPIECE * HSTRIDE) + (gg % per) * NROT + i * HSTRIDE + u


def _layernorm(x):
    m = jnp.mean(x, axis=-1, keepdims=True)
    d = x - m
    v = jnp.mean(d * d, axis=-1, keepdims=True)
    return d * jax.lax.rsqrt(v + EPS)


def _silu(x):
    return x * jax.nn.sigmoid(x)


def _dot(a, b):
    return jnp.dot(a, b, preferred_element_type=jnp.float32)


def _dot_nt(a, b):
    return jax.lax.dot_general(a, b, (((1,), (1,)), ((), ())), preferred_element_type=jnp.float32)


def _kernel(x_hbm, k_hbm, v_hbm, wq_hbm, wo_hbm, wr_hbm, wg_hbm, wu_hbm, wd_hbm, c_hbm, wm_hbm,
            out_ref,
            kbuf, vbuf, x_s, c_s, wr_s, wq_s, wo_s, wg_s, wu_s, wd_s, wm_s,
            q_s, mod_s, ksem, vsem, wsem, msem, *, dist, run, tail, fchunks, hrot, mrot):
    bf16 = jnp.bfloat16
    f32 = jnp.float32
    per = HSTRIDE // NROT

    def kv_pairs(g, sub):
        slot = sub % NSLOT
        p, q0 = g // per, (g % per) * NROT
        out = []
        for c0 in range(0, R, run * ROWS):
            for u in range(NROT):
                for c in range(c0, c0 + run * ROWS, ROWS):
                    src = pl.ds(sub * R + c, ROWS)
                    dst = pl.ds(c, ROWS)
                    out.append((
                        pltpu.make_async_copy(k_hbm.at[p, :, q0 + u, src], kbuf.at[slot, :, u, dst], ksem.at[slot]),
                        pltpu.make_async_copy(v_hbm.at[p, :, q0 + u, src], vbuf.at[slot, :, u, dst], vsem.at[slot])))
        return out

    def start_pairs(pairs):
        for kc, vc in pairs:
            kc.start(priority=0)
            if vc is not None:
                vc.start(priority=1)

    def tile_copies(src, dst, sem, rows, cols=None, rot=1):
        n, w = dst.shape
        cols = cols or w
        span = n // rot
        out = []
        for r in range(0, span, rows):
            for c0 in range(0, w, cols):
                for k in range(rot):
                    idx = (pl.ds(k * span + r, min(rows, span - r)), pl.ds(c0, cols))
                    out.append(pltpu.make_async_copy(src.at[idx], dst.at[idx], sem))
        return out

    def wait_all(buf, sem):
        pltpu.make_async_copy(buf, buf, sem).wait()

    wq_cp = tile_copies(wq_hbm, wq_s, wsem.at[2], 16, 1024, hrot)
    wm_cp = tile_copies(wm_hbm, wm_s, wsem.at[3], 16, 1024, hrot)
    wo_cp = tile_copies(wo_hbm, wo_s, wsem.at[4], 32, None, hrot)
    n_a = len(wq_cp) - len(wm_cp)
    head_a = list(zip(wq_cp, wm_cp + wo_cp[:n_a]))
    rest = wo_cp[n_a:]
    head_b = list(zip(rest[:len(rest) // 2], rest[len(rest) // 2:]))
    mlp_pairs = []
    slab_end = []
    for f, (f0, fn) in enumerate(fchunks):
        sl = pl.ds(f0, fn)
        cps = [tile_copies(src.at[sl], dst.at[sl], msem.at[f, t], 32)
               for t, (src, dst) in enumerate(((wg_hbm, wg_s), (wu_hbm, wu_s), (wd_hbm, wd_s)))]
        if mrot:
            flat = [cp for trio in zip(*cps) for cp in trio]
            mlp_pairs += list(zip(flat[0::2], flat[1::2] + [None] * (len(flat) % 2)))
        else:
            d = cps[2]
            dh = (len(d) + 1) // 2
            mlp_pairs += list(zip(cps[0] + d[:dh], cps[1] + d[dh:] + [None] * (2 * dh - len(d))))
        slab_end.append(len(mlp_pairs))
    n_mlp = len(mlp_pairs)


    def take_mlp(n):
        out = mlp_pairs[:n]
        del mlp_pairs[:n]
        return out

    x_cp = pltpu.make_async_copy(x_hbm, x_s, wsem.at[0])
    c_cp = pltpu.make_async_copy(c_hbm, c_s, wsem.at[1])
    wr_cp = pltpu.make_async_copy(wr_hbm, wr_s, wsem.at[5])
    x_cp.start(priority=0)
    c_cp.start(priority=1)
    wr_cp.start(priority=1)
    start_pairs(head_a)
    start_pairs(head_b)

    x_cp.wait()
    c_cp.wait()
    wait_all(wm_s, wsem.at[3])
    x = x_s[...].astype(f32)
    cc = _silu(c_s[...].astype(f32)).astype(bf16)
    mod = _dot(cc, wm_s[...])
    mod_s[...] = mod
    sa = mod[:, 0 * D:1 * D]
    ca = mod[:, 1 * D:2 * D]
    h = (_layernorm(x) * (1.0 + ca) + sa).astype(bf16)
    kv0 = kv_pairs(0, 0)
    start_pairs(kv0[:len(kv0) // 2])
    wait_all(wq_s, wsem.at[2])
    q = _dot(h, wq_s[...]) * (DH ** -0.5)
    start_pairs(kv0[len(kv0) // 2:])
    for b in range(B):
        for gg in range(GPB):
            for j in range(G):
                hd = _group_head(gg, j)
                q_s[b * GPB + gg, j:j + 1, :] = q[b:b + 1, hd * DH:(hd + 1) * DH]
    for s in range(1, dist):
        start_pairs(kv_pairs(0, s))

    wait_all(wo_s, wsem.at[4])
    row_s = jax.lax.broadcasted_iota(jnp.int32, (G, R), 0)
    row_o = jax.lax.broadcasted_iota(jnp.int32, (G, DH), 0)
    row_a = jax.lax.broadcasted_iota(jnp.int32, (G, D), 0)
    row_b = jax.lax.broadcasted_iota(jnp.int32, (B, D), 0)

    def substep(g, sub, qg, state, pairs_a, pairs_b):
        slot = sub % NSLOT
        wait_all(kbuf.at[slot], ksem.at[slot])
        s = None
        for j in range(G):
            sj = _dot_nt(qg, kbuf[slot, j // NROT, j % NROT])
            s = sj if s is None else jnp.where(row_s == j, sj, s)
        start_pairs(pairs_a)
        mcur = jnp.max(s, axis=-1, keepdims=True)
        if state is None:
            m = mcur
        else:
            m_old, l_old, o_old = state
            m = jnp.maximum(m_old, mcur)
        e = jnp.exp(s - m)
        l = jnp.sum(e, axis=-1, keepdims=True)
        eb = e.astype(bf16)
        wait_all(vbuf.at[slot], vsem.at[slot])
        o = None
        for j in range(G):
            oj = _dot(eb, vbuf[slot, j // NROT, j % NROT])
            o = oj if o is None else jnp.where(row_o == j, oj, o)
        start_pairs(pairs_b)
        if state is not None:
            alpha = jnp.exp(m_old - m)
            l = l + alpha * l_old
            o = o + alpha * o_old
        return m, l, o

    def group(g, attn, last):
        qg = q_s[g].astype(bf16)
        state = None
        for sub in range(NSUB):
            nxt = sub + dist
            if last and nxt >= NSUB:
                pa = take_mlp(tail[2 * (nxt - NSUB)])
                pb = take_mlp(tail[2 * (nxt - NSUB) + 1])
            else:
                pairs = kv_pairs(g + nxt // NSUB, nxt % NSUB)
                pa, pb = pairs[:len(pairs) // 2], pairs[len(pairs) // 2:]
            state = substep(g, sub, qg, state, pa, pb)
        _, l, o = state
        ob = (o / l).astype(bf16)
        gg = g % GPB
        h0 = (gg // per) * (NPIECE * HSTRIDE) + (gg % per) * NROT
        t = None
        for j in range(G):
            hd = h0 + (j // NROT) * HSTRIDE + j % NROT
            tj = _dot(ob, wo_s[pl.ds(pl.multiple_of(hd * DH, DH), DH), :])
            t = tj if t is None else jnp.where(row_a == j, tj, t)
        tsum = jnp.sum(t, axis=0, keepdims=True)
        return attn + jnp.where(row_b == g // GPB, tsum, 0.0)

    attn = jax.lax.fori_loop(0, NGRP - 1, lambda g, a: group(g, a, False), jnp.zeros((B, D), f32))
    attn = group(NGRP - 1, attn, True)

    start_pairs(take_mlp(tail[2 * dist]))
    wr_cp.wait()
    mod = mod_s[...]
    ga = mod[:, 2 * D:3 * D]
    sb = mod[:, 3 * D:4 * D]
    cb = mod[:, 4 * D:5 * D]
    gb = mod[:, 5 * D:6 * D]
    x1 = x_s[...].astype(f32) + ga * attn
    h2 = _layernorm(x1) * (1.0 + cb) + sb
    h2b = h2.astype(bf16)
    wr = wr_s[...].astype(f32)
    h2f = h2b.astype(f32)
    rp = h2f[:, 0:128] * wr[0:1, :]
    for j in range(1, D // 128):
        rp = rp + h2f[:, j * 128:(j + 1) * 128] * wr[j:j + 1, :]
    gate = gb * jax.nn.sigmoid(jnp.sum(rp, axis=-1, keepdims=True))
    base = x1 + gb * h2
    start_pairs(take_mlp(tail[2 * dist + 1]))
    y = None
    for f, (f0, fn) in enumerate(fchunks):
        sl = pl.ds(f0, fn)
        start_pairs(take_mlp(len(mlp_pairs) if f == len(fchunks) - 1 else tail[-1]))
        assert n_mlp - len(mlp_pairs) >= slab_end[f], "slab awaited before it was issued"
        for t, buf in enumerate((wg_s, wu_s, wd_s)):
            wait_all(buf.at[sl], msem.at[f, t])
        g = _silu(_dot_nt(h2b, wg_s[sl, :]))
        u = _dot_nt(h2b, wu_s[sl, :])
        yf = _dot((g * u).astype(bf16), wd_s[sl, :])
        y = yf if y is None else y + yf
    out_ref[...] = (base + gate * y).astype(out_ref.dtype)


def _build(dist=DIST, run=4, tail=(18, 18, 6, 6, 4, 5, 8), fslab=256, hrot=4, mrot=True):
    fchunks = tuple((f0, min(fslab, FF - f0)) for f0 in range(0, FF, fslab))
    bf16 = jnp.bfloat16
    hbm = pl.BlockSpec(memory_space=pltpu.HBM)
    scratch = [
        pltpu.VMEM((NSLOT, NPIECE, NROT, R, DH), bf16),
        pltpu.VMEM((NSLOT, NPIECE, NROT, R, DH), bf16),
        pltpu.VMEM((B, D), bf16),
        pltpu.VMEM((B, D), bf16),
        pltpu.VMEM((D // 128, 128), bf16),
        pltpu.VMEM((D, HQ * DH), bf16),
        pltpu.VMEM((HQ * DH, D), bf16),
        pltpu.VMEM((FF, D), bf16),
        pltpu.VMEM((FF, D), bf16),
        pltpu.VMEM((FF, D), bf16),
        pltpu.VMEM((D, 6 * D), bf16),
        pltpu.VMEM((NGRP, G, DH), jnp.float32),
        pltpu.VMEM((B, 6 * D), jnp.float32),
        pltpu.SemaphoreType.DMA((NSLOT,)),
        pltpu.SemaphoreType.DMA((NSLOT,)),
        pltpu.SemaphoreType.DMA((6,)),
        pltpu.SemaphoreType.DMA((len(fchunks), 3)),
    ]
    return pl.pallas_call(
        functools.partial(_kernel, dist=dist, run=run, tail=tail, fchunks=fchunks, hrot=hrot, mrot=mrot),
        out_shape=jax.ShapeDtypeStruct((B, D), bf16),
        in_specs=[hbm] * 11,
        out_specs=pl.BlockSpec(memory_space=pltpu.VMEM),
        scratch_shapes=scratch,
        compiler_params=pltpu.CompilerParams(vmem_limit_bytes=100 * 1024 * 1024),
    )


def _run(A_x, A_k_cache, A_v_cache, A_wq, A_wo, B_x, B_w_r, B_w_gate, B_w_up, B_w_down, c, w_mod, **kw):
    kv_shape = (B * HQ // (NPIECE * HSTRIDE), NPIECE, HSTRIDE, SK, DH)
    out = _build(**kw)(A_x.reshape(B, D), A_k_cache.reshape(kv_shape), A_v_cache.reshape(kv_shape),
                       A_wq, A_wo, B_w_r.reshape(D // 128, 128),
                       B_w_gate.T, B_w_up.T, B_w_down, c, w_mod)
    return out.reshape(B, 1, D)


@jax.jit
def pallas_adaLN_cond__gqa_block_cached__moe_arch_mod__decode_kernel(
    A_x: jax.Array,
    A_k_cache: jax.Array,
    A_v_cache: jax.Array,
    A_wq: jax.Array,
    A_wo: jax.Array,
    B_x: jax.Array,
    B_w_r: jax.Array,
    B_w_gate: jax.Array,
    B_w_up: jax.Array,
    B_w_down: jax.Array,
    c: jax.Array,
    w_mod: jax.Array,
):
    return _run(A_x, A_k_cache, A_v_cache, A_wq, A_wo, B_x, B_w_r, B_w_gate, B_w_up, B_w_down, c, w_mod)
```

```python
import jax
import jax.numpy as jnp
import jax.experimental.pallas as pl
import jax.experimental.pallas.tpu as pltpu

B, D, HQ, SK, DH, FF = 4, 512, 32, 8192, 128, 1376
EPS = 1e-5

NPIECE = 2
HSTRIDE = 8
NROT = 4
ROWS = 64
RUN = 1
G = NPIECE * NROT
R = SK // G
NSUB = SK // R
NGRP = B * HQ // G
GPB = HQ // G
PER = HSTRIDE // NROT
NSLOT = 4
DIST = 2

FSLAB = 256
SLABS = tuple((f0, min(FSLAB, FF - f0)) for f0 in range(0, FF, FSLAB))
TAIL_ISSUE = (18, 18, 6, 6, 4, 5, 8)

assert NSUB % NSLOT == 0 and DIST < NSLOT and len(TAIL_ISSUE) == 2 * DIST + 3


def _group_head(gg, j):
    return (gg // PER) * (NPIECE * HSTRIDE) + (gg % PER) * NROT + (j // NROT) * HSTRIDE + j % NROT


def _layernorm(x):
    m = jnp.mean(x, axis=-1, keepdims=True)
    d = x - m
    v = jnp.mean(d * d, axis=-1, keepdims=True)
    return d * jax.lax.rsqrt(v + EPS)


def _silu(x):
    return x * jax.nn.sigmoid(x)


def _dot(a, b):
    return jnp.dot(a, b, preferred_element_type=jnp.float32)


def _dot_nt(a, b):
    return jax.lax.dot_general(a, b, (((1,), (1,)), ((), ())), preferred_element_type=jnp.float32)


def _kernel(x_hbm, k_hbm, v_hbm, wq_hbm, wo_hbm, wr_hbm, wg_hbm, wu_hbm, wd_hbm, c_hbm, wm_hbm,
            out_ref,
            kbuf, vbuf, x_s, c_s, wr_s, wq_s, wo_s, wg_s, wu_s, wd_s, wm_s, q_s, mod_s,
            ksem, vsem, wsem, msem):
    bf16 = jnp.bfloat16
    f32 = jnp.float32

    def kv_pairs(g, sub):
        slot = sub % NSLOT
        p, q0 = g // PER, (g % PER) * NROT
        out = []
        for c0 in range(0, R, RUN * ROWS):
            for u in range(NROT):
                for c in range(c0, c0 + RUN * ROWS, ROWS):
                    src = pl.ds(sub * R + c, ROWS)
                    dst = pl.ds(c, ROWS)
                    out.append((
                        pltpu.make_async_copy(k_hbm.at[p, :, q0 + u, src], kbuf.at[slot, :, u, dst], ksem.at[slot]),
                        pltpu.make_async_copy(v_hbm.at[p, :, q0 + u, src], vbuf.at[slot, :, u, dst], vsem.at[slot])))
        return out

    def start_pairs(pairs):
        for a, b in pairs:
            a.start(priority=0)
            if b is not None:
                b.start(priority=1)

    def tile_copies(src, dst, sem, rows, cols=None, rot=1):
        n, w = dst.shape
        cols = cols or w
        span = n // rot
        out = []
        for r in range(0, span, rows):
            for c0 in range(0, w, cols):
                for k in range(rot):
                    idx = (pl.ds(k * span + r, min(rows, span - r)), pl.ds(c0, cols))
                    out.append(pltpu.make_async_copy(src.at[idx], dst.at[idx], sem))
        return out

    def wait_all(buf, sem):
        pltpu.make_async_copy(buf, buf, sem).wait()

    def split_queues(copies):
        return list(zip(copies[0::2], copies[1::2] + [None] * (len(copies) % 2)))

    wq_cp = tile_copies(wq_hbm, wq_s, wsem.at[3], 16, 1024, 4)
    wm_cp = tile_copies(wm_hbm, wm_s, wsem.at[4], 16, 1024, 4)
    wo_cp = tile_copies(wo_hbm, wo_s, wsem.at[5], 32, None, 4)
    n_a = len(wq_cp) - len(wm_cp)
    rest = wo_cp[n_a:]
    head_pairs = (list(zip(wq_cp, wm_cp + wo_cp[:n_a]))
                  + list(zip(rest[:len(rest) // 2], rest[len(rest) // 2:])))

    mlp_pairs = []
    slab_end = []
    for f, (f0, fn) in enumerate(SLABS):
        sl = pl.ds(f0, fn)
        cps = [tile_copies(src.at[sl], dst.at[sl], msem.at[f, t], 32)
               for t, (src, dst) in enumerate(((wg_hbm, wg_s), (wu_hbm, wu_s), (wd_hbm, wd_s)))]
        mlp_pairs += split_queues([cp for trio in zip(*cps) for cp in trio])
        slab_end.append(len(mlp_pairs))
    n_mlp = len(mlp_pairs)

    def take_mlp(n):
        out = mlp_pairs[:n]
        del mlp_pairs[:n]
        return out

    x_cp = pltpu.make_async_copy(x_hbm, x_s, wsem.at[0])
    c_cp = pltpu.make_async_copy(c_hbm, c_s, wsem.at[1])
    wr_cp = pltpu.make_async_copy(wr_hbm, wr_s, wsem.at[2])
    x_cp.start(priority=0)
    c_cp.start(priority=1)
    wr_cp.start(priority=1)
    start_pairs(head_pairs)

    x_cp.wait()
    c_cp.wait()
    wait_all(wm_s, wsem.at[4])
    x = x_s[...].astype(f32)
    cc = _silu(c_s[...].astype(f32)).astype(bf16)
    mod = _dot(cc, wm_s[...])
    mod_s[...] = mod
    sa = mod[:, 0 * D:1 * D]
    ca = mod[:, 1 * D:2 * D]
    h = (_layernorm(x) * (1.0 + ca) + sa).astype(bf16)
    kv0 = kv_pairs(0, 0)
    start_pairs(kv0[:len(kv0) // 2])
    wait_all(wq_s, wsem.at[3])
    q = _dot(h, wq_s[...]) * (DH ** -0.5)
    start_pairs(kv0[len(kv0) // 2:])
    for b in range(B):
        for gg in range(GPB):
            for j in range(G):
                hd = _group_head(gg, j)
                q_s[b * GPB + gg, j:j + 1, :] = q[b:b + 1, hd * DH:(hd + 1) * DH]
    for s in range(1, DIST):
        start_pairs(kv_pairs(0, s))
    wait_all(wo_s, wsem.at[5])

    row_s = jax.lax.broadcasted_iota(jnp.int32, (G, R), 0)
    row_o = jax.lax.broadcasted_iota(jnp.int32, (G, DH), 0)
    row_a = jax.lax.broadcasted_iota(jnp.int32, (G, D), 0)
    row_b = jax.lax.broadcasted_iota(jnp.int32, (B, D), 0)

    def substep(sub, qg, state, pairs_a, pairs_b):
        slot = sub % NSLOT
        wait_all(kbuf.at[slot], ksem.at[slot])
        s = None
        for j in range(G):
            sj = _dot_nt(qg, kbuf[slot, j // NROT, j % NROT])
            s = sj if s is None else jnp.where(row_s == j, sj, s)
        start_pairs(pairs_a)
        m = jnp.max(s, axis=-1, keepdims=True)
        if state is not None:
            m_old, l_old, o_old = state
            m = jnp.maximum(m_old, m)
        e = jnp.exp(s - m)
        l = jnp.sum(e, axis=-1, keepdims=True)
        eb = e.astype(bf16)
        wait_all(vbuf.at[slot], vsem.at[slot])
        o = None
        for j in range(G):
            oj = _dot(eb, vbuf[slot, j // NROT, j % NROT])
            o = oj if o is None else jnp.where(row_o == j, oj, o)
        start_pairs(pairs_b)
        if state is not None:
            alpha = jnp.exp(m_old - m)
            l = l + alpha * l_old
            o = o + alpha * o_old
        return m, l, o

    def group(g, attn, last):
        qg = q_s[g].astype(bf16)
        state = None
        for sub in range(NSUB):
            nxt = sub + DIST
            if last and nxt >= NSUB:
                pa = take_mlp(TAIL_ISSUE[2 * (nxt - NSUB)])
                pb = take_mlp(TAIL_ISSUE[2 * (nxt - NSUB) + 1])
            else:
                pairs = kv_pairs(g + nxt // NSUB, nxt % NSUB)
                pa, pb = pairs[:len(pairs) // 2], pairs[len(pairs) // 2:]
            state = substep(sub, qg, state, pa, pb)
        _, l, o = state
        ob = (o / l).astype(bf16)
        h0 = _group_head(g % GPB, 0)
        t = None
        for j in range(G):
            hd = h0 + (j // NROT) * HSTRIDE + j % NROT
            tj = _dot(ob, wo_s[pl.ds(pl.multiple_of(hd * DH, DH), DH), :])
            t = tj if t is None else jnp.where(row_a == j, tj, t)
        tsum = jnp.sum(t, axis=0, keepdims=True)
        return attn + jnp.where(row_b == g // GPB, tsum, 0.0)

    attn = jax.lax.fori_loop(0, NGRP - 1, lambda g, a: group(g, a, False), jnp.zeros((B, D), f32))
    attn = group(NGRP - 1, attn, True)

    start_pairs(take_mlp(TAIL_ISSUE[2 * DIST]))
    wr_cp.wait()
    mod = mod_s[...]
    ga = mod[:, 2 * D:3 * D]
    sb = mod[:, 3 * D:4 * D]
    cb = mod[:, 4 * D:5 * D]
    gb = mod[:, 5 * D:6 * D]
    x1 = x_s[...].astype(f32) + ga * attn
    h2 = _layernorm(x1) * (1.0 + cb) + sb
    h2b = h2.astype(bf16)
    wr = wr_s[...].astype(f32)
    h2f = h2b.astype(f32)
    rp = h2f[:, 0:128] * wr[0:1, :]
    for j in range(1, D // 128):
        rp = rp + h2f[:, j * 128:(j + 1) * 128] * wr[j:j + 1, :]
    gate = gb * jax.nn.sigmoid(jnp.sum(rp, axis=-1, keepdims=True))
    base = x1 + gb * h2
    start_pairs(take_mlp(TAIL_ISSUE[2 * DIST + 1]))
    y = None
    for f, (f0, fn) in enumerate(SLABS):
        sl = pl.ds(f0, fn)
        start_pairs(take_mlp(len(mlp_pairs) if f == len(SLABS) - 1 else TAIL_ISSUE[-1]))
        assert n_mlp - len(mlp_pairs) >= slab_end[f], "slab awaited before it was issued"
        for t, buf in enumerate((wg_s, wu_s, wd_s)):
            wait_all(buf.at[sl], msem.at[f, t])
        g = _silu(_dot_nt(h2b, wg_s[sl, :]))
        u = _dot_nt(h2b, wu_s[sl, :])
        yf = _dot((g * u).astype(bf16), wd_s[sl, :])
        y = yf if y is None else y + yf
    out_ref[...] = (base + gate * y).astype(out_ref.dtype)


def _run(A_x, A_k_cache, A_v_cache, A_wq, A_wo, B_x, B_w_r, B_w_gate, B_w_up, B_w_down, c, w_mod,
         interpret=False):
    del B_x
    bf16 = jnp.bfloat16
    hbm = pl.BlockSpec(memory_space=pltpu.HBM)
    scratch = [
        pltpu.VMEM((NSLOT, NPIECE, NROT, R, DH), bf16),
        pltpu.VMEM((NSLOT, NPIECE, NROT, R, DH), bf16),
        pltpu.VMEM((B, D), bf16),
        pltpu.VMEM((B, D), bf16),
        pltpu.VMEM((D // 128, 128), bf16),
        pltpu.VMEM((D, HQ * DH), bf16),
        pltpu.VMEM((HQ * DH, D), bf16),
        pltpu.VMEM((FF, D), bf16),
        pltpu.VMEM((FF, D), bf16),
        pltpu.VMEM((FF, D), bf16),
        pltpu.VMEM((D, 6 * D), bf16),
        pltpu.VMEM((NGRP, G, DH), jnp.float32),
        pltpu.VMEM((B, 6 * D), jnp.float32),
        pltpu.SemaphoreType.DMA((NSLOT,)),
        pltpu.SemaphoreType.DMA((NSLOT,)),
        pltpu.SemaphoreType.DMA((6,)),
        pltpu.SemaphoreType.DMA((len(SLABS), 3)),
    ]
    kv_view = (B * HQ // (NPIECE * HSTRIDE), NPIECE, HSTRIDE, SK, DH)
    out = pl.pallas_call(
        _kernel,
        out_shape=jax.ShapeDtypeStruct((B, D), bf16),
        in_specs=[hbm] * 11,
        out_specs=pl.BlockSpec(memory_space=pltpu.VMEM),
        scratch_shapes=scratch,
        compiler_params=pltpu.CompilerParams(vmem_limit_bytes=64 * 1024 * 1024),
        interpret=interpret,
    )(A_x.reshape(B, D), A_k_cache.reshape(kv_view), A_v_cache.reshape(kv_view), A_wq, A_wo,
      B_w_r.reshape(D // 128, 128), B_w_gate.T, B_w_up.T, B_w_down, c, w_mod)
    return out.reshape(B, 1, D)


@jax.jit
def pallas_adaLN_cond__gqa_block_cached__moe_arch_mod__decode_kernel(
    A_x: jax.Array,
    A_k_cache: jax.Array,
    A_v_cache: jax.Array,
    A_wq: jax.Array,
    A_wo: jax.Array,
    B_x: jax.Array,
    B_w_r: jax.Array,
    B_w_gate: jax.Array,
    B_w_up: jax.Array,
    B_w_down: jax.Array,
    c: jax.Array,
    w_mod: jax.Array,
):
    return _run(A_x, A_k_cache, A_v_cache, A_wq, A_wo, B_x, B_w_r, B_w_gate, B_w_up, B_w_down, c, w_mod)
```
